```python
import os as _os
_os.environ.setdefault("JAX_PLATFORMS", "cpu")
import jax
import jax.numpy as jnp

def _softmax(x, axis=-1):
    return jax.nn.softmax(x, axis=axis)
def _gelu(x):
    return jax.nn.gelu(x, approximate=True)
def _silu(x):
    return jax.nn.silu(x)
def _sigmoid(x):
    return jax.nn.sigmoid(x)
def _layernorm(x, axis=-1, eps=1e-5):
    m = jnp.mean(x, axis=axis, keepdims=True)
    v = jnp.var(x, axis=axis, keepdims=True)
    return (x - m) / jnp.sqrt(v + eps)
def _scatter_add(tgt, idx, src, axis=0):
    return tgt.at[idx].add(src)
def _segment_sum(src, seg, n):
    return jax.ops.segment_sum(src, seg, n)
class _Rng:
    def __init__(self, key):
        self._k = key
    def _next(self):
        self._k, sub = jax.random.split(self._k)
        return sub
    def normal(self, shape):
        return jax.random.normal(self._next(), shape, dtype=jnp.bfloat16)
    def randint(self, lo, hi, shape):
        return jax.random.randint(self._next(), shape, lo, hi, dtype=jnp.int32)
    def uniform(self, shape, lo=0.0, hi=1.0):
        return jax.random.uniform(self._next(), shape, jnp.bfloat16, lo, hi)
    def permutation(self, n):
        return jax.random.permutation(self._next(), n)


kernel_name = 'standalone__fft_conv__vision'

def setup_inputs():
    _rng = _Rng(jax.random.key(int.from_bytes(__import__("os").urandom(4), "little")))
    _w = (lambda a: (lambda t: t.astype(jnp.bfloat16) if jnp.issubdtype(t.dtype, jnp.floating) else t)(jnp.asarray(a)))
    H = W = 224
    C = 96
    K = 3
    return {
        "x": _w((lambda *s: _rng.normal(s) * 0.05)(1, H, W, C)),
        "w": _w((lambda *s: _rng.normal(s) * 0.05)(K, K, C, C)),
    }

def reference(x, w):
    B, H, W, C = x.shape
    K = w.shape[0]
    wp = jnp.pad(w, ((0, H - K), (0, W - K), (0, 0), (0, 0)))
    Xf = (lambda x, axes=(-2,-1): jnp.fft.rfft2(x.astype(jnp.float32), axes=axes))(x, axes=(1, 2))
    Wf = (lambda x, axes=(-2,-1): jnp.fft.rfft2(x.astype(jnp.float32), axes=axes))(wp, axes=(0, 1))
    Yf = jnp.einsum('bhwi,hwio->bhwo', Xf, Wf)
    y = (lambda x, s, axes=(-2,-1): jnp.fft.irfft2(x, s=s, axes=axes).astype(jnp.bfloat16))(Yf, (H, W), axes=(1, 2))
    return y
```

```python
import jax
import jax.numpy as jnp
import jax.experimental.pallas as pl
import jax.experimental.pallas.tpu as pltpu

H = 224
W = 224
C = 96
NTILES = H // 4
PHASES = ((2, 1), (4, 1), (8, 1), (14, 3))
assert sum(a * b for a, b in PHASES) == NTILES
HOLD = 22
MAXT = max(a for a, _ in PHASES)
NCHUNK = sum(b for _, b in PHASES)
LANES = ((0, 128), (128, W))

A1 = 2.0 / 3.0
B1 = 1.5
A2, B2 = A1 * A1, B1 * B1
NA = 2 * A2 * (A2 - B2)
NB = 2 * B2 * (B2 - A2)
f32 = jnp.float32
bf16 = jnp.bfloat16
u32 = jnp.uint32


def _to_u32(v):
    return pltpu.bitcast(v.astype(bf16), u32)


def _prep_weights(w_ref, lhs_ref, lhsl_ref):
    t = []
    for kh in range(3):
        c0 = jnp.concatenate([w_ref[kh, 0, 0:64, :], w_ref[kh, 1, 0:64, :]], axis=0).astype(f32)
        c1 = jnp.concatenate([w_ref[kh, 1, 64:96, :], w_ref[kh, 2]], axis=0).astype(f32)
        t.append((c0.T, c1.T))
    for c in range(2):
        g0, g1, g2 = t[2][c], t[1][c], t[0][c]
        ea = (g0 + A2 * g2) * (1.0 / NA)
        oa = g1 * (A1 / NA)
        eb = (g0 + B2 * g2) * (1.0 / NB)
        ob = g1 * (B1 / NB)
        mats = [g0, ea + oa, ea - oa, eb + ob, eb - ob, g2]
        for j in range(6):
            lhs_ref[j, :, c * 128:(c + 1) * 128] = _to_u32(mats[j])
    z = jnp.zeros((32, C), f32)
    l0, l1, l2 = [w_ref[kh, 0, 64:96, :].astype(f32) for kh in (2, 1, 0)]
    lhsl_ref[0:48, :] = _to_u32(jnp.concatenate([l0, l1, l2, z], axis=0).T)
    lhsl_ref[48:96, :] = _to_u32(jnp.concatenate([z, l0, l1, l2], axis=0).T)


def _input_transform(d0, d1, d2, d3, d4, d5):
    p = A2 * d2
    q = B2 * d2
    e = d4 - q
    e2 = d4 - p
    t0 = (d0 - p) + e
    p3 = A2 * d3
    q3 = B2 * d3
    o = d1 - p3
    o2 = d1 - q3
    t5 = (d5 - q3) + o
    bo = B1 * o
    ao2 = A1 * o2
    return [t0, e - bo, e + bo, e2 - ao2, e2 + ao2, t5]


def _build_tile(xbuf, r0, rhs):
    (ra, sa), (rb, sb) = rhs
    for g in range(6):
        ts = _input_transform(*[xbuf[r0 + l, 16 * g:16 * g + 16, :].astype(f32) for l in range(6)])
        for j in range(6):
            u1 = _to_u32(ts[j][:, 128:])
            u0 = _to_u32(ts[j][:, :128])
            h1 = jnp.concatenate([u1, u0[:, 96:]], axis=1)
            if g < 4:
                ra[sa + j, 8 * g:8 * g + 8, :] = u0
                rb[sb + j, 8 * g:8 * g + 8, :] = h1
            for kw in (1, 2):
                off = 32 + 48 * (kw - 1) + 8 * g
                ra[sa + j, off:off + 8, kw:] = pltpu.roll(u0, kw, 1)[:, kw:]
                ra[sa + j, off:off + 8, :kw] = pltpu.roll(h1, 32 + kw, 1)[:, :kw]
                rb[sb + j, off:off + 8, :] = pltpu.roll(h1, kw, 1)


def _mm_tile(xbuf, r0, rhs, zero, lhs_ref, lhsl_ref, obuf, after):
    for n, (lo, hi) in enumerate(LANES):
        ref, off = rhs[n]

        def m(j):
            r = pltpu.bitcast(ref[zero + (off + j)], bf16)
            return jnp.dot(pltpu.bitcast(lhs_ref[j], bf16), r, preferred_element_type=f32)[:, :hi - lo]

        def direct(l0):
            r = jnp.concatenate([xbuf[r0 + l, 64:96, lo:hi] for l in range(l0, l0 + 4)], axis=0)
            return jnp.dot(pltpu.bitcast(lhsl_ref[...], bf16), r, preferred_element_type=f32)

        def store(k, val):
            obuf[r0 + k, :, lo:hi] = val.astype(bf16)

        m1, m2 = m(1), m(2)
        s, d = m1 + m2, m1 - m2
        m3, m4 = m(3), m(4)
        s2, d2 = m3 + m4, m3 - m4
        la = direct(0)
        m0 = m(0)
        ad = A1 * d
        bd = B1 * d2
        store(0, (m0 + la[:96]) + (s + s2))
        store(1, (ad + bd) + la[96:])
        lb = direct(2)
        m5 = m(5)
        store(2, (A2 * s + B2 * s2) + lb[:96])
        store(3, (A2 * ad + B2 * bd) + (m5 + lb[96:]))
        if after is not None:
            after(lo, hi)


def _kernel(x_hbm, w_hbm, o_hbm, xbuf, obuf, wbuf, lhs_ref, lhsl_ref, isem, osem, msem, *rhs_refs):
    w_cp = pltpu.make_async_copy(w_hbm, wbuf, msem.at[0])
    h_cp = pltpu.make_async_copy(x_hbm.at[pl.ds(H - 2, 2)], xbuf.at[pl.ds(0, 2)], msem.at[1])
    f_cp = pltpu.make_async_copy(x_hbm.at[pl.ds(0, 4)], xbuf.at[pl.ds(2, 4)], msem.at[2])

    def in_rows(c, tstart, ntiles):
        return pltpu.make_async_copy(x_hbm.at[pl.ds(4 * tstart + 4, 4 * ntiles)],
                                     xbuf.at[pl.ds(4 * tstart + 6, 4 * ntiles)], isem.at[c])

    def out_rows(r0, n):
        return pltpu.make_async_copy(obuf.at[pl.ds(r0, n)], o_hbm.at[pl.ds(r0, n)], osem.at[0])

    w_cp.start()
    h_cp.start()
    f_cp.start()
    c = 0
    t = 0
    for tpb, cnt in PHASES:
        for _ in range(cnt):
            in_rows(c, t, tpb if t + tpb < NTILES else tpb - 1).start()
            c += 1
            t += tpb

    w_cp.wait()
    _prep_weights(wbuf, lhs_ref, lhsl_ref)
    h_cp.wait()
    f_cp.wait()
    _build_tile(xbuf, 0, ((rhs_refs[0], 0), (rhs_refs[0], 6)))

    def block(c, tpb, cnt, c0, tb, last_phase):
        slots = [((r, 0), (r, 6)) for r in rhs_refs[:tpb]]
        if tpb > 2:
            slots[tpb - 1] = ((rhs_refs[tpb - 1], 0), (rhs_refs[0], 12))
        zero = jax.lax.shift_right_logical(c, 12)
        it = c - c0
        t0 = tb + it * tpb if cnt > 1 else tb
        if last_phase:
            @pl.when(it < cnt - 1)
            def _():
                in_rows(c, t0, tpb).wait()

            @pl.when(it == cnt - 1)
            def _():
                in_rows(c, t0, tpb - 1).wait()
        else:
            in_rows(c0, t0, tpb).wait()
        base = 4 * t0
        for k in range(tpb):
            rn = base + 4 * (k + 1)
            if k == tpb - 1 and last_phase:
                rn = jnp.where(it == cnt - 1, 0, rn)
            _build_tile(xbuf, rn, slots[(k + 1) % tpb])
            split = last_phase and k == tpb - 1

            def after(lo, hi, k=k):
                pltpu.make_async_copy(obuf.at[pl.ds(base + 4 * k, 4), :, lo:hi],
                                      o_hbm.at[pl.ds(base + 4 * k, 4), :, lo:hi], osem.at[0]).start()

            _mm_tile(xbuf, base + 4 * k, slots[k], zero, lhs_ref, lhsl_ref, obuf, after if split else None)
            if split:
                assert tb + k >= HOLD
            elif tb + k >= HOLD:
                out_rows(base + 4 * k, 4).start()
            elif tb + (cnt - 1) * tpb + k >= HOLD:
                @pl.when(t0 + k >= HOLD)
                def _():
                    out_rows(base + 4 * k, 4).start()
            if tb <= HOLD - 1 - k <= tb + (cnt - 1) * tpb and (HOLD - 1 - k - tb) % tpb == 0:
                @pl.when(t0 + k == HOLD - 1)
                def _():
                    out_rows(0, 4 * HOLD).start()

    def body(c, carry):
        c0 = 0
        tb = 0
        for pi, (tpb, cnt) in enumerate(PHASES):
            last_phase = pi == len(PHASES) - 1
            assert last_phase or cnt == 1

            @pl.when(jnp.logical_and(c >= c0, c < c0 + cnt))
            def _(tpb=tpb, cnt=cnt, c0=c0, tb=tb, last_phase=last_phase):
                block(c, tpb, cnt, c0, tb, last_phase)

            c0 += cnt
            tb += tpb * cnt
        return carry

    jax.lax.fori_loop(0, NCHUNK, body, 0)
    out_rows(0, H).wait()


@jax.jit
def pallas_standalone__fft_conv__vision_kernel(x, w):
    xt = jnp.transpose(x, (0, 1, 3, 2)).reshape(H, C, W)
    out = pl.pallas_call(
        _kernel,
        in_specs=[pl.BlockSpec(memory_space=pl.ANY), pl.BlockSpec(memory_space=pl.ANY)],
        out_specs=pl.BlockSpec(memory_space=pl.ANY),
        out_shape=jax.ShapeDtypeStruct((H, C, W), bf16),
        scratch_shapes=[
            pltpu.VMEM((H + 2, C, W), bf16),
            pltpu.VMEM((H, C, W), bf16),
            pltpu.VMEM((3, 3, C, C), bf16),
            pltpu.VMEM((6, C // 2, 256), u32),
            pltpu.VMEM((C, 128), u32),
            pltpu.SemaphoreType.DMA((NCHUNK,)),
            pltpu.SemaphoreType.DMA((1,)),
            pltpu.SemaphoreType.DMA((3,)),
        ] + [pltpu.VMEM((18 if k == 0 else 12, 128, 128), u32) for k in range(MAXT)],
        compiler_params=pltpu.CompilerParams(
            vmem_limit_bytes=64 * 1024 * 1024,
            disable_bounds_checks=True,
            disable_semaphore_checks=True,
        ),
    )(xt, w)
    return jnp.transpose(out.reshape(1, H, C, W), (0, 1, 3, 2))
```

```python
import jax
import jax.numpy as jnp
import jax.experimental.pallas as pl
import jax.experimental.pallas.tpu as pltpu

H = 224
W = 224
C = 96
NTILES = H // 4
BLOCKS = (2, 4, 8, 16, 26)
assert sum(BLOCKS) == NTILES
HOLD = 24
CATCH = 2 * HOLD - 3
JG = 2
LANES = ((0, 128), (128, W))

A1 = 2.0 / 3.0
B1 = 1.5
A2, B2 = A1 * A1, B1 * B1
NA = 2 * A2 * (A2 - B2)
NB = 2 * B2 * (B2 - A2)
f32 = jnp.float32
bf16 = jnp.bfloat16
u32 = jnp.uint32


def _to_u32(v):
    return pltpu.bitcast(v.astype(bf16), u32)


def _prep_weights(w_ref, lhs_ref, lhsl_ref):
    t = []
    for kh in range(3):
        c0 = jnp.concatenate([w_ref[kh, 0, 0:64, :], w_ref[kh, 1, 0:64, :]], axis=0).astype(f32)
        c1 = jnp.concatenate([w_ref[kh, 1, 64:96, :], w_ref[kh, 2]], axis=0).astype(f32)
        t.append((c0.T, c1.T))
    for c in range(2):
        g0, g1, g2 = t[2][c], t[1][c], t[0][c]
        ea = (g0 + A2 * g2) * (1.0 / NA)
        oa = g1 * (A1 / NA)
        eb = (g0 + B2 * g2) * (1.0 / NB)
        ob = g1 * (B1 / NB)
        mats = [g0, ea + oa, ea - oa, eb + ob, eb - ob, g2]
        for j in range(6):
            lhs_ref[j, :, c * 128:(c + 1) * 128] = _to_u32(mats[j])
    z = jnp.zeros((32, C), f32)
    l0, l1, l2 = [w_ref[kh, 0, 64:96, :].astype(f32) for kh in (2, 1, 0)]
    lhsl_ref[0:48, :] = _to_u32(jnp.concatenate([l0, l1, l2, z], axis=0).T)
    lhsl_ref[48:96, :] = _to_u32(jnp.concatenate([z, l0, l1, l2], axis=0).T)


def _input_transform(d0, d1, d2, d3, d4, d5):
    p = A2 * d2
    q = B2 * d2
    e = d4 - q
    e2 = d4 - p
    t0 = (d0 - p) + e
    p3 = A2 * d3
    q3 = B2 * d3
    o = d1 - p3
    o2 = d1 - q3
    t5 = (d5 - q3) + o
    bo = B1 * o
    ao2 = A1 * o2
    return [t0, e - bo, e + bo, e2 - ao2, e2 + ao2, t5]


def _build_tile(xbuf, r0, rhs):
    (ra, sa), (rb, sb) = rhs
    for g in range(6):
        tl = _input_transform(*[xbuf[r0 + l, 16 * g:16 * g + 16, :].astype(f32) for l in range(6)])
        for j in range(0, 6, JG):
            ts = jnp.stack(tl[j:j + JG])
            u1 = _to_u32(ts[:, :, 128:])
            u0 = _to_u32(ts[:, :, :128])
            h1 = jnp.concatenate([u1, u0[:, :, 96:]], axis=2)
            ja, jb = slice(sa + j, sa + j + JG), slice(sb + j, sb + j + JG)
            if g < 4:
                ra[ja, 8 * g:8 * g + 8, :] = u0
                rb[jb, 8 * g:8 * g + 8, :] = h1
            for kw in (1, 2):
                off = 32 + 48 * (kw - 1) + 8 * g
                ra[ja, off:off + 8, kw:] = pltpu.roll(u0, kw, 2)[:, :, kw:]
                ra[ja, off:off + 8, :kw] = pltpu.roll(h1, 32 + kw, 2)[:, :, :kw]
                rb[jb, off:off + 8, :] = pltpu.roll(h1, kw, 2)


def _mm_tile(xbuf, r0, rhs, zero, lhs_ref, lhsl_ref, obuf, after):
    for n, (lo, hi) in enumerate(LANES):
        ref, off = rhs[n]

        def m(j):
            r = pltpu.bitcast(ref[zero + (off + j)], bf16)
            return jnp.dot(pltpu.bitcast(lhs_ref[j], bf16), r, preferred_element_type=f32)[:, :hi - lo]

        def direct(l0):
            r = jnp.concatenate([xbuf[r0 + l, 64:96, lo:hi] for l in range(l0, l0 + 4)], axis=0)
            return jnp.dot(pltpu.bitcast(lhsl_ref[...], bf16), r, preferred_element_type=f32)

        def store(k, val):
            obuf[r0 + k, :, lo:hi] = val.astype(bf16)

        m1, m2 = m(1), m(2)
        s, d = m1 + m2, m1 - m2
        m3, m4 = m(3), m(4)
        s2, d2 = m3 + m4, m3 - m4
        la = direct(0)
        m0 = m(0)
        ad = A1 * d
        bd = B1 * d2
        store(0, (m0 + la[:96]) + (s + s2))
        store(1, (ad + bd) + la[96:])
        lb = direct(2)
        m5 = m(5)
        store(2, (A2 * s + B2 * s2) + lb[:96])
        store(3, (A2 * ad + B2 * bd) + (m5 + lb[96:]))
        if after is not None:
            after(lo, hi)


def _kernel(x_hbm, w_hbm, o_hbm, xbuf, obuf, lhs_ref, lhsl_ref, isem, osem, msem, *rest):
    rhs_refs, wbuf = rest[:-1], rest[-1]
    w_cp = pltpu.make_async_copy(w_hbm, wbuf, msem.at[0])
    h_cp = pltpu.make_async_copy(x_hbm.at[pl.ds(H - 2, 2)], xbuf.at[pl.ds(0, 2)], msem.at[1])
    f_cp = pltpu.make_async_copy(x_hbm.at[pl.ds(0, 4)], xbuf.at[pl.ds(2, 4)], msem.at[2])
    in_cps = []
    t0 = 0
    for b, nt in enumerate(BLOCKS):
        r0 = 4 * t0 + 4
        nrows = min(4 * nt, H - 2 - r0)
        in_cps.append(pltpu.make_async_copy(x_hbm.at[pl.ds(r0, nrows)], xbuf.at[pl.ds(r0 + 2, nrows)],
                                            isem.at[b]))
        t0 += nt

    def out_tiles(t, n):
        for q in range(2 * n):
            rows = pl.ds(4 * t + 2 * q, 2)
            pltpu.make_async_copy(obuf.at[rows], o_hbm.at[rows], osem.at[0]).start(priority=q % 2)

    def out_last(lo, hi):
        rows = pl.ds(H - 4, 4)
        pltpu.make_async_copy(obuf.at[rows, :, lo:hi], o_hbm.at[rows, :, lo:hi], osem.at[0]).start()

    w_cp.start()
    h_cp.start()
    f_cp.start()
    for cp in in_cps:
        cp.start()

    w_cp.wait()
    _prep_weights(wbuf, lhs_ref, lhsl_ref)
    h_cp.wait()
    f_cp.wait()
    xbuf[H:H + 2] = xbuf[0:2]
    _build_tile(xbuf, 0, ((rhs_refs[0], 0), (rhs_refs[0], 6)))

    def main(zero):
        t0 = 0
        for b, nt in enumerate(BLOCKS):
            slots = [((r, 0), (r, 6)) for r in rhs_refs[:nt]]
            if nt > 2:
                slots[nt - 1] = ((rhs_refs[nt - 1], 0), (rhs_refs[0], 12))
            in_cps[b].wait()
            for k in range(nt):
                t = t0 + k
                last = t == NTILES - 1
                if not last:
                    _build_tile(xbuf, 4 * t + 4, slots[(k + 1) % nt])
                _mm_tile(xbuf, 4 * t, slots[k], zero, lhs_ref, lhsl_ref, obuf, out_last if last else None)
                if t == HOLD - 1:
                    out_tiles(0, 1)
                if HOLD - 1 <= t < CATCH:
                    out_tiles(2 * (t - HOLD + 1) + 1, 2)
                elif CATCH <= t and not last:
                    out_tiles(t, 1)
            t0 += nt

    def body(c, carry):
        @pl.when(c == 0)
        def _():
            main(jax.lax.shift_right_logical(c, 12))
        return carry

    jax.lax.fori_loop(0, 2, body, 0)
    pltpu.make_async_copy(obuf, o_hbm, osem.at[0]).wait()


@jax.jit
def pallas_standalone__fft_conv__vision_kernel(x, w):
    xt = jnp.transpose(x, (0, 1, 3, 2)).reshape(H, C, W)
    out = pl.pallas_call(
        _kernel,
        in_specs=[pl.BlockSpec(memory_space=pl.ANY), pl.BlockSpec(memory_space=pl.ANY)],
        out_specs=pl.BlockSpec(memory_space=pl.ANY),
        out_shape=jax.ShapeDtypeStruct((H, C, W), bf16),
        scratch_shapes=[
            pltpu.VMEM((H + 2, C, W), bf16),
            pltpu.VMEM((H, C, W), bf16),
            pltpu.VMEM((6, C // 2, 256), u32),
            pltpu.VMEM((C, 128), u32),
            pltpu.SemaphoreType.DMA((len(BLOCKS),)),
            pltpu.SemaphoreType.DMA((1,)),
            pltpu.SemaphoreType.DMA((3,)),
        ] + [pltpu.VMEM((18 if k == 0 else 12, 128, 128), u32) for k in range(max(BLOCKS))] + [
            pltpu.VMEM((3, 3, C, C), bf16),
        ],
        compiler_params=pltpu.CompilerParams(
            vmem_limit_bytes=64 * 1024 * 1024,
            disable_bounds_checks=True,
            disable_semaphore_checks=True,
        ),
    )(xt, w)
    return jnp.transpose(out.reshape(1, H, C, W), (0, 1, 3, 2))
```

```python
import jax
import jax.numpy as jnp
import jax.experimental.pallas as pl
import jax.experimental.pallas.tpu as pltpu

H = 224
W = 224
C = 96
NTILES = H // 4
BLOCKS = (2, 4, 8, 16, 26)
assert sum(BLOCKS) == NTILES
HOLD = 24
CATCH = 2 * HOLD - 3
JG = 2
LANES = ((0, 128), (128, W))

A1 = 2.0 / 3.0
B1 = 1.5
A2, B2 = A1 * A1, B1 * B1
NA = 2 * A2 * (A2 - B2)
NB = 2 * B2 * (B2 - A2)
f32 = jnp.float32
bf16 = jnp.bfloat16
u32 = jnp.uint32


def _to_u32(v):
    return pltpu.bitcast(v.astype(bf16), u32)


def _prep_weights(w_ref, lhs_ref, lhsl_ref):
    t = []
    for kh in range(3):
        c0 = jnp.concatenate([w_ref[kh, 0, 0:64, :], w_ref[kh, 1, 0:64, :]], axis=0).astype(f32)
        c1 = jnp.concatenate([w_ref[kh, 1, 64:96, :], w_ref[kh, 2]], axis=0).astype(f32)
        t.append((c0.T, c1.T))
    for c in range(2):
        g0, g1, g2 = t[2][c], t[1][c], t[0][c]
        ea = (g0 + A2 * g2) * (1.0 / NA)
        oa = g1 * (A1 / NA)
        eb = (g0 + B2 * g2) * (1.0 / NB)
        ob = g1 * (B1 / NB)
        mats = [g0, ea + oa, ea - oa, eb + ob, eb - ob, g2]
        for j in range(6):
            lhs_ref[j, :, c * 128:(c + 1) * 128] = _to_u32(mats[j])
    z = jnp.zeros((32, C), f32)
    l0, l1, l2 = [w_ref[kh, 0, 64:96, :].astype(f32) for kh in (2, 1, 0)]
    lhsl_ref[0:48, :] = _to_u32(jnp.concatenate([l0, l1, l2, z], axis=0).T)
    lhsl_ref[48:96, :] = _to_u32(jnp.concatenate([z, l0, l1, l2], axis=0).T)


def _input_transform(d0, d1, d2, d3, d4, d5):
    p = A2 * d2
    q = B2 * d2
    e = d4 - q
    e2 = d4 - p
    t0 = (d0 - p) + e
    p3 = A2 * d3
    q3 = B2 * d3
    o = d1 - p3
    o2 = d1 - q3
    t5 = (d5 - q3) + o
    bo = B1 * o
    ao2 = A1 * o2
    return [t0, e - bo, e + bo, e2 - ao2, e2 + ao2, t5]


def _build_tile(xbuf, r0, rhs):
    (ra, sa), (rb, sb) = rhs
    ja, jb = slice(sa, sa + 6), slice(sb, sb + 6)
    for g in range(6):
        d = xbuf[r0:r0 + 6, 16 * g:16 * g + 16, :].astype(f32)
        tl = _input_transform(*[d[l] for l in range(6)])
        vals = []
        for j in range(0, 6, JG):
            t = jnp.stack(tl[j:j + JG])
            u1 = _to_u32(t[:, :, 128:])
            u0 = _to_u32(t[:, :, :128])
            h1 = jnp.concatenate([u1, u0[:, :, 96:]], axis=2)
            v = [u0, h1]
            for kw in (1, 2):
                v += [pltpu.roll(u0, kw, 2), pltpu.roll(h1, 32 + kw, 2), pltpu.roll(h1, kw, 2)]
            vals.append(v)
        v = [jnp.concatenate(q, axis=0) for q in zip(*vals)]
        if g < 4:
            ra[ja, 8 * g:8 * g + 8, :] = v[0]
            rb[jb, 8 * g:8 * g + 8, :] = v[1]
        for kw in (1, 2):
            off = 32 + 48 * (kw - 1) + 8 * g
            ra[ja, off:off + 8, kw:] = v[3 * kw - 1][:, :, kw:]
            ra[ja, off:off + 8, :kw] = v[3 * kw][:, :, :kw]
            rb[jb, off:off + 8, :] = v[3 * kw + 1]


def _mm_tile(xbuf, r0, rhs, zero, lhs_ref, lhsl_ref, obuf, after):
    for n, (lo, hi) in enumerate(LANES):
        ref, off = rhs[n]

        def m(j):
            r = pltpu.bitcast(ref[zero + (off + j)], bf16)
            return jnp.dot(pltpu.bitcast(lhs_ref[j], bf16), r, preferred_element_type=f32)[:, :hi - lo]

        def direct(l0):
            r = xbuf[r0 + l0:r0 + l0 + 4, 64:96, lo:hi].reshape(128, hi - lo)
            return jnp.dot(pltpu.bitcast(lhsl_ref[...], bf16), r, preferred_element_type=f32)

        def store(k, val):
            obuf[r0 + k, :, lo:hi] = val.astype(bf16)

        m1, m2 = m(1), m(2)
        s, d = m1 + m2, m1 - m2
        m3, m4 = m(3), m(4)
        s2, d2 = m3 + m4, m3 - m4
        la = direct(0)
        m0 = m(0)
        ad = A1 * d
        bd = B1 * d2
        store(0, (m0 + la[:96]) + (s + s2))
        store(1, (ad + bd) + la[96:])
        lb = direct(2)
        m5 = m(5)
        store(2, (A2 * s + B2 * s2) + lb[:96])
        store(3, (A2 * ad + B2 * bd) + (m5 + lb[96:]))
        if after is not None:
            after(lo, hi)


def _kernel(x_hbm, w_hbm, o_hbm, xbuf, obuf, lhs_ref, lhsl_ref, isem, osem, msem, *rest):
    rhs_refs, wbuf = rest[:-1], rest[-1]
    w_cp = pltpu.make_async_copy(w_hbm, wbuf, msem.at[0])
    h_cp = pltpu.make_async_copy(x_hbm.at[pl.ds(H - 2, 2)], xbuf.at[pl.ds(0, 2)], msem.at[1])
    f_cp = pltpu.make_async_copy(x_hbm.at[pl.ds(0, 4)], xbuf.at[pl.ds(2, 4)], msem.at[2])
    in_cps = []
    t0 = 0
    for b, nt in enumerate(BLOCKS):
        r0 = 4 * t0 + 4
        nrows = min(4 * nt, H - 2 - r0)
        in_cps.append(pltpu.make_async_copy(x_hbm.at[pl.ds(r0, nrows)], xbuf.at[pl.ds(r0 + 2, nrows)],
                                            isem.at[b]))
        t0 += nt

    def out_tiles(t, n):
        for q in range(2 * n):
            rows = pl.ds(4 * t + 2 * q, 2)
            pltpu.make_async_copy(obuf.at[rows], o_hbm.at[rows], osem.at[0]).start(priority=q % 2)

    def out_last(lo, hi):
        rows = pl.ds(H - 4, 4)
        pltpu.make_async_copy(obuf.at[rows, :, lo:hi], o_hbm.at[rows, :, lo:hi], osem.at[0]).start()

    w_cp.start()
    h_cp.start()
    f_cp.start()
    for cp in in_cps:
        cp.start()

    w_cp.wait()
    _prep_weights(wbuf, lhs_ref, lhsl_ref)
    h_cp.wait()
    f_cp.wait()
    xbuf[H:H + 2] = xbuf[0:2]
    _build_tile(xbuf, 0, ((rhs_refs[0], 0), (rhs_refs[0], 6)))

    def main(zero):
        t0 = 0
        for b, nt in enumerate(BLOCKS):
            slots = [((r, 0), (r, 6)) for r in rhs_refs[:nt]]
            if nt > 2:
                slots[nt - 1] = ((rhs_refs[nt - 1], 0), (rhs_refs[0], 12))
            in_cps[b].wait()
            for k in range(nt):
                t = t0 + k
                last = t == NTILES - 1
                if not last:
                    _build_tile(xbuf, 4 * t + 4, slots[(k + 1) % nt])
                _mm_tile(xbuf, 4 * t, slots[k], zero, lhs_ref, lhsl_ref, obuf, out_last if last else None)
                if t == HOLD - 1:
                    out_tiles(0, 1)
                if HOLD - 1 <= t < CATCH:
                    out_tiles(2 * (t - HOLD + 1) + 1, 2)
                elif CATCH <= t and not last:
                    out_tiles(t, 1)
            t0 += nt

    def body(c, carry):
        @pl.when(c == 0)
        def _():
            main(jax.lax.shift_right_logical(c, 12))
        return carry

    jax.lax.fori_loop(0, 2, body, 0)
    pltpu.make_async_copy(obuf, o_hbm, osem.at[0]).wait()


@jax.jit
def pallas_standalone__fft_conv__vision_kernel(x, w):
    xt = jnp.transpose(x, (0, 1, 3, 2)).reshape(H, C, W)
    out = pl.pallas_call(
        _kernel,
        in_specs=[pl.BlockSpec(memory_space=pl.ANY), pl.BlockSpec(memory_space=pl.ANY)],
        out_specs=pl.BlockSpec(memory_space=pl.ANY),
        out_shape=jax.ShapeDtypeStruct((H, C, W), bf16),
        scratch_shapes=[
            pltpu.VMEM((H + 2, C, W), bf16),
            pltpu.VMEM((H, C, W), bf16),
            pltpu.VMEM((6, C // 2, 256), u32),
            pltpu.VMEM((C, 128), u32),
            pltpu.SemaphoreType.DMA((len(BLOCKS),)),
            pltpu.SemaphoreType.DMA((1,)),
            pltpu.SemaphoreType.DMA((3,)),
        ] + [pltpu.VMEM((18 if k == 0 else 12, 128, 128), u32) for k in range(max(BLOCKS))] + [
            pltpu.VMEM((3, 3, C, C), bf16),
        ],
        compiler_params=pltpu.CompilerParams(
            vmem_limit_bytes=64 * 1024 * 1024,
            disable_bounds_checks=True,
            disable_semaphore_checks=True,
        ),
    )(xt, w)
    return jnp.transpose(out.reshape(1, H, C, W), (0, 1, 3, 2))
```

```python
import jax
import jax.numpy as jnp
import jax.experimental.pallas as pl
import jax.experimental.pallas.tpu as pltpu

H = 224
W = 224
C = 96
NTILES = H // 4
BLOCKS = (2, 4, 8, 16, 26)
assert sum(BLOCKS) == NTILES
HOLD = 24
CATCH = 2 * HOLD - 3
JG = 2
LANES = ((0, 128), (128, W))

A1 = 2.0 / 3.0
B1 = 1.5
A2, B2 = A1 * A1, B1 * B1
NA = 2 * A2 * (A2 - B2)
NB = 2 * B2 * (B2 - A2)
f32 = jnp.float32
bf16 = jnp.bfloat16
u32 = jnp.uint32


def _to_u32(v):
    return pltpu.bitcast(v.astype(bf16), u32)


def _prep_weights(w_ref, lhs_ref, lhsl_ref):
    t = []
    for kh in range(3):
        c0 = jnp.concatenate([w_ref[kh, 0, 0:64, :], w_ref[kh, 1, 0:64, :]], axis=0).astype(f32)
        c1 = jnp.concatenate([w_ref[kh, 1, 64:96, :], w_ref[kh, 2]], axis=0).astype(f32)
        t.append((c0.T, c1.T))
    for c in range(2):
        g0, g1, g2 = t[2][c], t[1][c], t[0][c]
        ea = (g0 + A2 * g2) * (1.0 / NA)
        oa = g1 * (A1 / NA)
        eb = (g0 + B2 * g2) * (1.0 / NB)
        ob = g1 * (B1 / NB)
        mats = [g0, ea + oa, ea - oa, eb + ob, eb - ob, g2]
        for j in range(6):
            lhs_ref[j, :, c * 128:(c + 1) * 128] = _to_u32(mats[j])
    z = jnp.zeros((32, C), f32)
    l0, l1, l2 = [w_ref[kh, 0, 64:96, :].astype(f32) for kh in (2, 1, 0)]
    lhsl_ref[0:48, :] = _to_u32(jnp.concatenate([l0, l1, l2, z], axis=0).T)
    lhsl_ref[48:96, :] = _to_u32(jnp.concatenate([z, l0, l1, l2], axis=0).T)


def _input_transform(d0, d1, d2, d3, d4, d5):
    p = A2 * d2
    q = B2 * d2
    e = d4 - q
    e2 = d4 - p
    t0 = (d0 - p) + e
    p3 = A2 * d3
    q3 = B2 * d3
    o = d1 - p3
    o2 = d1 - q3
    t5 = (d5 - q3) + o
    bo = B1 * o
    ao2 = A1 * o2
    return [t0, e - bo, e + bo, e2 - ao2, e2 + ao2, t5]


def _build_tile(xbuf, r0, rhs):
    (ra, sa), (rb, sb) = rhs
    ja, jb = slice(sa, sa + 6), slice(sb, sb + 6)
    for g in range(6):
        d = xbuf[r0:r0 + 6, 16 * g:16 * g + 16, :].astype(f32)
        tl = _input_transform(*[d[l] for l in range(6)])
        vals = []
        for j in range(0, 6, JG):
            t = jnp.stack(tl[j:j + JG])
            u1 = _to_u32(t[:, :, 128:])
            u0 = _to_u32(t[:, :, :128])
            h1 = jnp.concatenate([u1, u0[:, :, 96:]], axis=2)
            v = [u0, h1]
            for kw in (1, 2):
                v += [pltpu.roll(u0, kw, 2), pltpu.roll(h1, 32 + kw, 2), pltpu.roll(h1, kw, 2)]
            vals.append(v)
        v = [jnp.concatenate(q, axis=0) for q in zip(*vals)]
        if g < 4:
            ra[ja, 8 * g:8 * g + 8, :] = v[0]
            rb[jb, 8 * g:8 * g + 8, :] = v[1]
        for kw in (1, 2):
            off = 32 + 48 * (kw - 1) + 8 * g
            ra[ja, off:off + 8, kw:] = v[3 * kw - 1][:, :, kw:]
            ra[ja, off:off + 8, :kw] = v[3 * kw][:, :, :kw]
            rb[jb, off:off + 8, :] = v[3 * kw + 1]


def _mm_tile(xbuf, r0, rhs, zero, lhs_ref, lhsl_ref, obuf, after):
    for n, (lo, hi) in enumerate(LANES):
        ref, off = rhs[n]

        def m(j):
            r = pltpu.bitcast(ref[zero + (off + j)], bf16)
            return jnp.dot(pltpu.bitcast(lhs_ref[j], bf16), r, preferred_element_type=f32)[:, :hi - lo]

        def direct(l0):
            r = xbuf[r0 + l0:r0 + l0 + 4, 64:96, lo:hi].reshape(128, hi - lo)
            return jnp.dot(pltpu.bitcast(lhsl_ref[...], bf16), r, preferred_element_type=f32)

        def store(k, val):
            obuf[r0 + k, :, lo:hi] = val.astype(bf16)

        m1, m2 = m(1), m(2)
        s, d = m1 + m2, m1 - m2
        m3, m4 = m(3), m(4)
        s2, d2 = m3 + m4, m3 - m4
        la = direct(0)
        m0 = m(0)
        ad = A1 * d
        bd = B1 * d2
        store(0, (m0 + la[:96]) + (s + s2))
        store(1, (ad + bd) + la[96:])
        lb = direct(2)
        m5 = m(5)
        store(2, (A2 * s + B2 * s2) + lb[:96])
        store(3, (A2 * ad + B2 * bd) + (m5 + lb[96:]))
        if after is not None:
            after(n).start()


def _kernel(x_hbm, w_hbm, o_hbm, xbuf, obuf, lhs_ref, lhsl_ref, isem, osem, msem, *rest):
    rhs_refs, wbuf = rest[:-1], rest[-1]
    w_cp = pltpu.make_async_copy(w_hbm, wbuf, msem.at[0])
    h_cp = pltpu.make_async_copy(x_hbm.at[pl.ds(H - 2, 2)], xbuf.at[pl.ds(0, 2)], msem.at[1])
    f_cp = pltpu.make_async_copy(x_hbm.at[pl.ds(0, 4)], xbuf.at[pl.ds(2, 4)], msem.at[2])
    in_cps = []
    t0 = 0
    for b, nt in enumerate(BLOCKS):
        r0 = 4 * t0 + 4
        nrows = min(4 * nt, H - 2 - r0)
        in_cps.append(pltpu.make_async_copy(x_hbm.at[pl.ds(r0, nrows)], xbuf.at[pl.ds(r0 + 2, nrows)],
                                            isem.at[b]))
        t0 += nt

    def out_tiles(t, n):
        for q in range(2 * n):
            rows = pl.ds(4 * t + 2 * q, 2)
            pltpu.make_async_copy(obuf.at[rows], o_hbm.at[rows], osem.at[0]).start(priority=q % 2)

    def out_last(n):
        rows, (lo, hi) = pl.ds(H - 4, 4), LANES[n]
        return pltpu.make_async_copy(obuf.at[rows, :, lo:hi], o_hbm.at[rows, :, lo:hi], osem.at[1 + n])

    w_cp.start()
    h_cp.start()
    f_cp.start()
    for cp in in_cps:
        cp.start()

    w_cp.wait()
    _prep_weights(wbuf, lhs_ref, lhsl_ref)
    h_cp.wait()
    f_cp.wait()
    xbuf[H:H + 2] = xbuf[0:2]
    _build_tile(xbuf, 0, ((rhs_refs[0], 0), (rhs_refs[0], 6)))

    def main(zero):
        t0 = 0
        for b, nt in enumerate(BLOCKS):
            slots = [((r, 0), (r, 6)) for r in rhs_refs[:nt]]
            if nt > 2:
                slots[nt - 1] = ((rhs_refs[nt - 1], 0), (rhs_refs[0], 12))
            in_cps[b].wait()
            for k in range(nt):
                t = t0 + k
                last = t == NTILES - 1
                if not last:
                    _build_tile(xbuf, 4 * t + 4, slots[(k + 1) % nt])
                _mm_tile(xbuf, 4 * t, slots[k], zero, lhs_ref, lhsl_ref, obuf, out_last if last else None)
                if t == HOLD - 1:
                    out_tiles(0, 1)
                if HOLD - 1 <= t < CATCH:
                    out_tiles(2 * (t - HOLD + 1) + 1, 2)
                elif CATCH <= t and not last:
                    out_tiles(t, 1)
            t0 += nt

    def body(c, carry):
        @pl.when(c == 0)
        def _():
            main(jax.lax.shift_right_logical(c, 12))
        return carry

    jax.lax.fori_loop(0, 2, body, 0)
    pltpu.make_async_copy(obuf.at[pl.ds(0, H - 4)], o_hbm.at[pl.ds(0, H - 4)], osem.at[0]).wait()
    out_last(0).wait()
    out_last(1).wait()


@jax.jit
def pallas_standalone__fft_conv__vision_kernel(x, w):
    xt = jnp.transpose(x, (0, 1, 3, 2)).reshape(H, C, W)
    out = pl.pallas_call(
        _kernel,
        in_specs=[pl.BlockSpec(memory_space=pl.ANY), pl.BlockSpec(memory_space=pl.ANY)],
        out_specs=pl.BlockSpec(memory_space=pl.ANY),
        out_shape=jax.ShapeDtypeStruct((H, C, W), bf16),
        scratch_shapes=[
            pltpu.VMEM((H + 2, C, W), bf16),
            pltpu.VMEM((H, C, W), bf16),
            pltpu.VMEM((6, C // 2, 256), u32),
            pltpu.VMEM((C, 128), u32),
            pltpu.SemaphoreType.DMA((len(BLOCKS),)),
            pltpu.SemaphoreType.DMA((3,)),
            pltpu.SemaphoreType.DMA((3,)),
        ] + [pltpu.VMEM((18 if k == 0 else 12, 128, 128), u32) for k in range(max(BLOCKS))] + [
            pltpu.VMEM((3, 3, C, C), bf16),
        ],
        compiler_params=pltpu.CompilerParams(
            vmem_limit_bytes=64 * 1024 * 1024,
            disable_semaphore_checks=True,
        ),
    )(xt, w)
    return jnp.transpose(out.reshape(1, H, C, W), (0, 1, 3, 2))
```

```python
import jax
import jax.numpy as jnp
import jax.experimental.pallas as pl
import jax.experimental.pallas.tpu as pltpu

H = 224
W = 224
C = 96
NTILES = H // 4
BLOCKS = (2, 4, 8, 16, 26)
assert sum(BLOCKS) == NTILES
HOLD = 24
CATCH = 2 * HOLD - 3
JG = 2
LANES = ((0, 128), (128, W))

A1 = 2.0 / 3.0
B1 = 1.5
A2, B2 = A1 * A1, B1 * B1
NA = 2 * A2 * (A2 - B2)
NB = 2 * B2 * (B2 - A2)
f32 = jnp.float32
bf16 = jnp.bfloat16
u32 = jnp.uint32


def _to_u32(v):
    return pltpu.bitcast(v.astype(bf16), u32)


def _prep_weights(w_ref, lhs_ref, lhsl_ref):
    t = []
    for kh in range(3):
        c0 = jnp.concatenate([w_ref[kh, 0, 0:64, :], w_ref[kh, 1, 0:64, :]], axis=0).astype(f32)
        c1 = jnp.concatenate([w_ref[kh, 1, 64:96, :], w_ref[kh, 2]], axis=0).astype(f32)
        t.append((c0.T, c1.T))
    for c in range(2):
        g0, g1, g2 = t[2][c], t[1][c], t[0][c]
        ea = (g0 + A2 * g2) * (1.0 / NA)
        oa = g1 * (A1 / NA)
        eb = (g0 + B2 * g2) * (1.0 / NB)
        ob = g1 * (B1 / NB)
        mats = [g0, ea + oa, ea - oa, eb + ob, eb - ob, g2]
        for j in range(6):
            lhs_ref[j, :, c * 128:(c + 1) * 128] = _to_u32(mats[j])
    z = jnp.zeros((32, C), f32)
    l0, l1, l2 = [w_ref[kh, 0, 64:96, :].astype(f32) for kh in (2, 1, 0)]
    lhsl_ref[0:48, :] = _to_u32(jnp.concatenate([l0, l1, l2, z], axis=0).T)
    lhsl_ref[48:96, :] = _to_u32(jnp.concatenate([z, l0, l1, l2], axis=0).T)


def _input_transform(d0, d1, d2, d3, d4, d5):
    p = A2 * d2
    q = B2 * d2
    e = d4 - q
    e2 = d4 - p
    t0 = (d0 - p) + e
    p3 = A2 * d3
    q3 = B2 * d3
    o = d1 - p3
    o2 = d1 - q3
    t5 = (d5 - q3) + o
    bo = B1 * o
    ao2 = A1 * o2
    return [t0, e - bo, e + bo, e2 - ao2, e2 + ao2, t5]


def _build_tile(xbuf, r0, rhs):
    (ra, sa), (rb, sb) = rhs
    ja, jb = slice(sa, sa + 6), slice(sb, sb + 6)
    for g in range(6):
        d = xbuf[r0:r0 + 6, 16 * g:16 * g + 16, :].astype(f32)
        tl = _input_transform(*[d[l] for l in range(6)])
        vals = []
        for j in range(0, 6, JG):
            t = jnp.stack(tl[j:j + JG])
            u1 = _to_u32(t[:, :, 128:])
            u0 = _to_u32(t[:, :, :128])
            h1 = jnp.concatenate([u1, u0[:, :, 96:]], axis=2)
            v = [u0, h1]
            for kw in (1, 2):
                v += [pltpu.roll(u0, kw, 2), pltpu.roll(h1, 32 + kw, 2), pltpu.roll(h1, kw, 2)]
            vals.append(v)
        v = [jnp.concatenate(q, axis=0) for q in zip(*vals)]
        if g < 4:
            ra[ja, 8 * g:8 * g + 8, :] = v[0]
            rb[jb, 8 * g:8 * g + 8, :] = v[1]
        for kw in (1, 2):
            off = 32 + 48 * (kw - 1) + 8 * g
            ra[ja, off:off + 8, kw:] = v[3 * kw - 1][:, :, kw:]
            ra[ja, off:off + 8, :kw] = v[3 * kw][:, :, :kw]
            rb[jb, off:off + 8, :] = v[3 * kw + 1]


def _mm_tile(xbuf, r0, rhs, zero, lhs_ref, lhsl_ref, obuf, after):
    for n, (lo, hi) in enumerate(LANES):
        ref, off = rhs[n]

        def m(j):
            r = pltpu.bitcast(ref[zero + (off + j)], bf16)
            return jnp.dot(pltpu.bitcast(lhs_ref[j], bf16), r, preferred_element_type=f32)[:, :hi - lo]

        def direct(l0):
            r = xbuf[r0 + l0:r0 + l0 + 4, 64:96, lo:hi].reshape(128, hi - lo)
            return jnp.dot(pltpu.bitcast(lhsl_ref[...], bf16), r, preferred_element_type=f32)

        def store(k, val):
            obuf[r0 + k, :, lo:hi] = val.astype(bf16)

        m1, m2 = m(1), m(2)
        s, d = m1 + m2, m1 - m2
        m3, m4 = m(3), m(4)
        s2, d2 = m3 + m4, m3 - m4
        la = direct(0)
        m0 = m(0)
        ad = A1 * d
        bd = B1 * d2
        store(0, (m0 + la[:96]) + (s + s2))
        store(1, (ad + bd) + la[96:])
        lb = direct(2)
        m5 = m(5)
        store(2, (A2 * s + B2 * s2) + lb[:96])
        store(3, (A2 * ad + B2 * bd) + (m5 + lb[96:]))
        if after is not None:
            after(n).start()


def _kernel(x_hbm, w_hbm, o_hbm, xbuf, obuf, lhs_ref, lhsl_ref, isem, osem, msem, *rest):
    rhs_refs, wbuf = rest[:-1], rest[-1]
    w_cp = pltpu.make_async_copy(w_hbm, wbuf, msem.at[0])
    h_cp = pltpu.make_async_copy(x_hbm.at[pl.ds(H - 2, 2)], xbuf.at[pl.ds(0, 2)], msem.at[1])
    f_cp = pltpu.make_async_copy(x_hbm.at[pl.ds(0, 4)], xbuf.at[pl.ds(2, 4)], msem.at[2])
    in_cps = []
    t0 = 0
    for b, nt in enumerate(BLOCKS):
        r0 = 4 * t0 + 4
        nrows = min(4 * nt, H - 2 - r0)
        in_cps.append(pltpu.make_async_copy(x_hbm.at[pl.ds(r0, nrows)], xbuf.at[pl.ds(r0 + 2, nrows)],
                                            isem.at[b]))
        t0 += nt

    def out_tiles(t, n):
        for q in range(2 * n):
            rows = pl.ds(4 * t + 2 * q, 2)
            pltpu.make_async_copy(obuf.at[rows], o_hbm.at[rows], osem.at[0]).start(priority=q % 2)

    def out_last(n):
        rows, (lo, hi) = pl.ds(H - 4, 4), LANES[n]
        return pltpu.make_async_copy(obuf.at[rows, :, lo:hi], o_hbm.at[rows, :, lo:hi], osem.at[1 + n])

    w_cp.start()
    h_cp.start()
    f_cp.start()
    for cp in in_cps:
        cp.start()

    w_cp.wait()
    _prep_weights(wbuf, lhs_ref, lhsl_ref)
    h_cp.wait()
    f_cp.wait()
    xbuf[H:H + 2] = xbuf[0:2]
    _build_tile(xbuf, 0, ((rhs_refs[0], 0), (rhs_refs[0], 6)))

    def main(zero):
        t0 = 0
        for b, nt in enumerate(BLOCKS):
            slots = [((r, 0), (r, 6)) for r in rhs_refs[:nt]]
            if nt > 2:
                slots[nt - 1] = ((rhs_refs[nt - 1], 0), (rhs_refs[0], 12))
            in_cps[b].wait()
            for k in range(nt):
                t = t0 + k
                last = t == NTILES - 1
                if not last:
                    _build_tile(xbuf, 4 * t + 4, slots[(k + 1) % nt])
                _mm_tile(xbuf, 4 * t, slots[k], zero, lhs_ref, lhsl_ref, obuf, out_last if last else None)
                if t == HOLD - 1:
                    out_tiles(0, 1)
                if HOLD - 1 <= t < CATCH:
                    out_tiles(2 * (t - HOLD + 1) + 1, 2)
                elif CATCH <= t and not last:
                    out_tiles(t, 1)
            t0 += nt

    def body(c, carry):
        @pl.when(c == 0)
        def _():
            main(jax.lax.shift_right_logical(c, 12))
        return carry

    jax.lax.fori_loop(0, 2, body, 0)
    pltpu.make_async_copy(obuf.at[pl.ds(0, H - 4)], o_hbm.at[pl.ds(0, H - 4)], osem.at[0]).wait()
    out_last(0).wait()
    out_last(1).wait()


def _compiler_params():
    try:
        return pltpu.CompilerParams(vmem_limit_bytes=64 * 1024 * 1024, disable_semaphore_checks=True)
    except TypeError:
        return pltpu.CompilerParams(vmem_limit_bytes=64 * 1024 * 1024)


@jax.jit
def pallas_standalone__fft_conv__vision_kernel(x, w):
    xt = jnp.transpose(x, (0, 1, 3, 2)).reshape(H, C, W)
    out = pl.pallas_call(
        _kernel,
        in_specs=[pl.BlockSpec(memory_space=pl.ANY), pl.BlockSpec(memory_space=pl.ANY)],
        out_specs=pl.BlockSpec(memory_space=pl.ANY),
        out_shape=jax.ShapeDtypeStruct((H, C, W), bf16),
        scratch_shapes=[
            pltpu.VMEM((H + 2, C, W), bf16),
            pltpu.VMEM((H, C, W), bf16),
            pltpu.VMEM((6, C // 2, 256), u32),
            pltpu.VMEM((C, 128), u32),
            pltpu.SemaphoreType.DMA((len(BLOCKS),)),
            pltpu.SemaphoreType.DMA((3,)),
            pltpu.SemaphoreType.DMA((3,)),
        ] + [pltpu.VMEM((18 if k == 0 else 12, 128, 128), u32) for k in range(max(BLOCKS))] + [
            pltpu.VMEM((3, 3, C, C), bf16),
        ],
        compiler_params=_compiler_params(),
    )(xt, w)
    return jnp.transpose(out.reshape(1, H, C, W), (0, 1, 3, 2))
```
